```python
import jax
import jax.numpy as jnp

def _softmax(x, axis=-1):
    return jax.nn.softmax(x, axis=axis)
def _gelu(x):
    return jax.nn.gelu(x, approximate=True)
def _silu(x):
    return jax.nn.silu(x)
def _sigmoid(x):
    return jax.nn.sigmoid(x)
def _layernorm(x, axis=-1, eps=1e-5):
    m = jnp.mean(x, axis=axis, keepdims=True)
    v = jnp.var(x, axis=axis, keepdims=True)
    return (x - m) / jnp.sqrt(v + eps)
def _scatter_add(tgt, idx, src, axis=0):
    return tgt.at[idx].add(src)
def _segment_sum(src, seg, n):
    return jax.ops.segment_sum(src, seg, n)
class _Rng:
    def __init__(self, key):
        self._k = key
    def _next(self):
        self._k, sub = jax.random.split(self._k)
        return sub
    def normal(self, shape):
        return jax.random.normal(self._next(), shape, dtype=jnp.bfloat16)
    def randint(self, lo, hi, shape):
        return jax.random.randint(self._next(), shape, lo, hi, dtype=jnp.int32)
    def uniform(self, shape, lo=0.0, hi=1.0):
        return jax.random.uniform(self._next(), shape, jnp.bfloat16, lo, hi)
    def permutation(self, n):
        return jax.random.permutation(self._next(), n)


kernel_name = 'sequential_preLN__compressed_kv_cla__moe_arch_mod__prompt'

def setup_inputs():
    _rng = _Rng(jax.random.key(int.from_bytes(__import__("os").urandom(4), "little")))
    _w = (lambda a: (lambda t: t.astype(jnp.bfloat16) if jnp.issubdtype(t.dtype, jnp.floating) else t)(jnp.asarray(a)))
    def _A_setup():
        B, H, Sq, Sk, D, M = 1, 32, 2048, 2048, 128, 1024
        Dc = 4 * D
        return {
            "x": _w((lambda *s: _rng.normal(s) * 0.05)(B, Sq, M)),
            "c_kv": _w((lambda *s: _rng.normal(s) * 0.05)(B, Sk, Dc)),
            "w_q": _w((lambda *s: _rng.normal(s) * 0.05)(M, H, D) * (M ** -0.5)),
            "w_uk": _w((lambda *s: _rng.normal(s) * 0.05)(Dc, H, D) * (Dc ** -0.5)),
            "w_uv": _w((lambda *s: _rng.normal(s) * 0.05)(Dc, H, D) * (Dc ** -0.5)),
            "w_o": _w((lambda *s: _rng.normal(s) * 0.05)(H, D, M) * ((H * D) ** -0.5)),
        }
    _A_in = _A_setup()

    def _B_setup():
        B, S, D, F, C = 1, 2048, 1024, 3584, 2
        return {
            "x": _w((lambda *s: _rng.normal(s) * 0.05)(B, S, D)),
            "w_r": _w((lambda *s: _rng.normal(s) * 0.05)(D)),
            "w_gate": _w((lambda *s: _rng.normal(s) * 0.05)(D, F)),
            "w_up": _w((lambda *s: _rng.normal(s) * 0.05)(D, F)),
            "w_down": _w((lambda *s: _rng.normal(s) * 0.05)(F, D)),
        }
    _B_in = _B_setup()

    return {
        "A_x": _A_in["x"],
        "A_c_kv": _A_in["c_kv"],
        "A_w_q": _A_in["w_q"],
        "A_w_uk": _A_in["w_uk"],
        "A_w_uv": _A_in["w_uv"],
        "A_w_o": _A_in["w_o"],
        "B_x": _B_in["x"],
        "B_w_r": _B_in["w_r"],
        "B_w_gate": _B_in["w_gate"],
        "B_w_up": _B_in["w_up"],
        "B_w_down": _B_in["w_down"],
    }

def reference(A_x, A_c_kv, A_w_q, A_w_uk, A_w_uv, A_w_o, B_x, B_w_r, B_w_gate, B_w_up, B_w_down):
    def _A_ref(x, c_kv, w_q, w_uk, w_uv, w_o):
        B, Sq, M = x.shape[0], x.shape[1], x.shape[2]
        Sk = c_kv.shape[1]
        H, D = w_q.shape[1], w_q.shape[2]
        q = jnp.einsum("bqm,mhd->bhqd", x, w_q)
        k = jnp.einsum("bkc,chd->bhkd", c_kv, w_uk)
        v = jnp.einsum("bkc,chd->bhkd", c_kv, w_uv)
        scores = jnp.einsum("bhqd,bhkd->bhqk", q, k) * (D ** -0.5)
        off = Sk - Sq
        qi = jnp.arange(Sq)[:, None]
        kj = jnp.arange(Sk)[None, :]
        cmask = kj <= (qi + off)
        scores = jnp.where(cmask[None, None], scores, -1e9)
        p = _softmax(scores, axis=-1)
        ctx = jnp.einsum("bhqk,bhkd->bhqd", p, v)
        return jnp.einsum("bhqd,hdm->bqm", ctx, w_o)

    def _B_ref(x, w_r, w_gate, w_up, w_down):
        B, S, D = x.shape
        C = 2
        r = x @ w_r
        idx = jnp.argsort(-r, axis=-1)[:, :C]
        idx_e = jnp.repeat(idx.reshape(B, C, 1), D, axis=2)
        x_sel = jnp.take_along_axis(x, idx_e, axis=1)
        g = _silu(x_sel @ w_gate)
        u = x_sel @ w_up
        y = (g * u) @ w_down
        r_sel = _sigmoid(jnp.take_along_axis(r, idx, axis=1))
        y = y * r_sel.reshape(B, C, 1)
        b_off = (jnp.arange(B) * S).reshape(B, 1)
        flat_idx = (idx + b_off).reshape(B * C)
        zero = (x * 0.0).reshape(B * S, D)
        upd = _scatter_add(zero, flat_idx, y.reshape(B * C, D), axis=0)
        return x + upd.reshape(B, S, D)

    x = A_x
    h = x + _A_ref(_layernorm(x, axis=-1), A_c_kv, A_w_q, A_w_uk, A_w_uv, A_w_o)
    h2 = h + _B_ref(_layernorm(h, axis=-1), B_w_r, B_w_gate, B_w_up, B_w_down)
    return h2
```

```python
import os
import numpy as np
import jax
import jax.numpy as jnp
import jax.experimental.pallas as pl
import jax.experimental.pallas.tpu as pltpu

_S, _M, _H, _D, _DC, _F = 2048, 1024, 32, 128, 512, 3584
_NP = _H // 2
_BQ = 256
_EPS = 1e-5
_NT = (((1,), (1,)), ((), ()))
_F32, _BF16 = jnp.float32, jnp.bfloat16
_SCHED = os.environ.get("SCHED", "0")
_DIAG = int(os.environ.get("DIAG", 0))
_RC = int(os.environ.get("RC", 512))
_SKEW = int(os.environ.get("SKEW", 1))
_RB = int(os.environ.get("RB", 256))


def _unpack_pair(w32):
    lo = pltpu.bitcast(w32 << 16, _F32).astype(_BF16)
    hi = pltpu.bitcast(w32 & np.uint32(0xFFFF0000), _F32).astype(_BF16)
    return pltpu.bitcast(jnp.concatenate([lo, hi], axis=1), jnp.uint32)


def _ld(ref, r0, rows, cols=slice(None), lead=None):
    rs = pl.ds(r0 // 2, rows // 2) if isinstance(r0, int) else pl.ds(pl.multiple_of(r0 // 2, rows // 2), rows // 2)
    v = ref[rs, cols] if lead is None else ref[lead, rs, cols]
    return pltpu.bitcast(v, _BF16)


def _st(ref, r0, val, cols=slice(None), lead=None):
    rows = val.shape[0]
    rs = pl.ds(r0 // 2, rows // 2) if isinstance(r0, int) else pl.ds(pl.multiple_of(r0 // 2, rows // 2), rows // 2)
    v = pltpu.bitcast(val.astype(_BF16), jnp.uint32)
    if lead is None:
        ref[rs, cols] = v
    else:
        ref[lead, rs, cols] = v


def _recip(l):
    r = pl.reciprocal(l, approx=True)
    return r + r * (1.0 - l * r)


def _rb(v):
    return v.astype(_BF16).astype(_F32)


def _schedule():
    nq = _S // _BQ
    nr = _S // _RC
    P = [("k", r) for r in range(nr)] + [("v", r) for r in range(nr)] + [("q", r) for r in range(nr)]
    A_seq = [("a", hh, qb) for hh in range(2) for qb in reversed(range(nq))]
    A_int = [("a", hh, qb) for qb in reversed(range(nq)) for hh in range(2)]
    if _SCHED == "0":
        return P + A_seq
    if _SCHED == "1":
        return P + A_int
    if _SCHED == "2":
        out = []
        slots = len(A_int)
        pos = [int(round(x)) for x in np.linspace(4, slots, len(P))]
        for j, a in enumerate(A_int):
            out.append(a)
            out += [p for p, q in zip(P, pos) if q == j + 1]
        return out
    if _SCHED == "3":
        out = list(A_int[:8])
        rest = A_int[8:]
        for j, a in enumerate(rest):
            out.append(a)
            out += P[(len(P) * j) // len(rest):(len(P) * (j + 1)) // len(rest)]
        return out
    if _SCHED == "4":
        out = P[:len(P) // 2] + A_int[:8]
        rest = A_int[8:]
        P2 = P[len(P) // 2:]
        for j, a in enumerate(rest):
            out.append(a)
            out += P2[(len(P2) * j) // len(rest):(len(P2) * (j + 1)) // len(rest)]
        return out
    if _SCHED == "5":
        A = [("a", hh, qb) for qb in range(nq) for hh in range(2)]
        out = []
        for j, a in enumerate(A):
            out.append(a)
            out += P[(len(P) * j) // len(A):(len(P) * (j + 1)) // len(A)]
        return out
    if _SCHED == "6":
        out = []
        for j, a in enumerate(A_int):
            out.append(a)
            out += P[(len(P) * j) // len(A_int):(len(P) * (j + 1)) // len(A_int)]
        return out
    raise ValueError


def _kernel(x_hbm, ckv_hbm, wq_hbm, wk_hbm, wv_hbm, wo_hbm, wr_ref, wg_hbm, wu_hbm, wd_hbm,
            out_hbm,
            x_v, ckv_v, ln_v, wq_v, wk_v, wv_v, wo_v, wg_v, wu_v, wd_v,
            wqb, wkb, wvb, q_v, k_v, v_v, ctx_v, out_v, r_v, acc_v,
            sem_a, sem_w, sem_o):
    wq32 = wq_hbm.bitcast(jnp.uint32)
    wk32 = wk_hbm.bitcast(jnp.uint32)
    wv32 = wv_hbm.bitcast(jnp.uint32)
    x_hbm, ckv_hbm, wo_hbm, wg_hbm, wu_hbm, wd_hbm, out_hbm = [
        t.bitcast(jnp.uint32) for t in (x_hbm, ckv_hbm, wo_hbm, wg_hbm, wu_hbm, wd_hbm, out_hbm)]

    cp_ckv = pltpu.make_async_copy(ckv_hbm, ckv_v, sem_a.at[0])
    cp_x = pltpu.make_async_copy(x_hbm, x_v, sem_a.at[1])
    cp_wo = pltpu.make_async_copy(wo_hbm, wo_v, sem_a.at[2])
    cp_wg = pltpu.make_async_copy(wg_hbm, wg_v, sem_a.at[3])
    cp_wu = pltpu.make_async_copy(wu_hbm, wu_v, sem_a.at[4])
    cp_wd = pltpu.make_async_copy(wd_hbm, wd_v, sem_a.at[5])

    def cp_wq(i):
        return pltpu.make_async_copy(wq32.at[:, i, :], wq_v.at[i], sem_w.at[0, i])

    def cp_wk(i):
        return pltpu.make_async_copy(wk32.at[:, i, :], wk_v.at[i], sem_w.at[1, i])

    def cp_wv(i):
        return pltpu.make_async_copy(wv32.at[:, i, :], wv_v.at[i], sem_w.at[2, i])

    cp_ckv.start()
    cp_wk(0).start()
    cp_wv(0).start()
    cp_x.start()
    cp_wq(0).start()

    qscale = np.float32(_D ** -0.5 * np.log2(np.e))

    def proj(kind, r, slot):
        r0 = r * _RC
        if kind == "k":
            _st(k_v, r0, jnp.dot(_ld(ckv_v, r0, _RC), _ld(wkb, 0, _DC), preferred_element_type=_F32), lead=slot)
        elif kind == "v":
            _st(v_v, r0, jnp.dot(_ld(ckv_v, r0, _RC), _ld(wvb, 0, _DC), preferred_element_type=_F32), lead=slot)
        else:
            q = jnp.dot(_ld(ln_v, r0, _RC), _ld(wqb, 0, _M), preferred_element_type=_F32)
            _st(q_v, r0, q * qscale, lead=slot)

    hb = _BQ // 2

    def attn1(i, slot, hh, qb):
        hs = slice(hh * _D, (hh + 1) * _D)
        q = _ld(q_v, qb * _BQ, _BQ, hs, slot)
        ri = jax.lax.broadcasted_iota(jnp.int32, (hb, hb), 0)
        ci = jax.lax.broadcasted_iota(jnp.int32, (hb, hb), 1)
        keep = ci <= ri
        n = qb * _BQ + hb
        s1 = jax.lax.dot_general(q, _ld(k_v, 0, n, hs, slot), _NT, preferred_element_type=_F32)
        s2 = jax.lax.dot_general(q[hb:], _ld(k_v, n, hb, hs, slot), _NT, preferred_element_type=_F32)
        su = jnp.where(keep, s1[:hb, n - hb:], -1e9)
        if qb > 0:
            su = jnp.concatenate([s1[:hb, :n - hb], su], axis=1)
        sl = jnp.concatenate([s1[hb:], jnp.where(keep, s2, -1e9)], axis=1)
        return su, sl, jnp.max(su, axis=1, keepdims=True), jnp.max(sl, axis=1, keepdims=True)

    def attn2(i, slot, hh, qb, st):
        hs = slice(hh * _D, (hh + 1) * _D)
        su, sl, mu, ml = st
        n = qb * _BQ + hb
        pu = jnp.exp2(su - mu)
        pl_ = jnp.exp2(sl - ml)
        lu = jnp.sum(pu, axis=1, keepdims=True)
        ll = jnp.sum(pl_, axis=1, keepdims=True)
        p1 = jnp.concatenate([pu, pl_[:, :n]], axis=0).astype(_BF16)
        o = jnp.dot(p1, _ld(v_v, 0, n, hs, slot), preferred_element_type=_F32)
        o2 = jnp.dot(pl_[:, n:].astype(_BF16), _ld(v_v, n, hb, hs, slot), preferred_element_type=_F32)
        _st(ctx_v, qb * _BQ, o[:hb] * _recip(lu), hs, i)
        _st(ctx_v, qb * _BQ + hb, (o[hb:] + o2) * _recip(ll), hs, i)

    def run_sched(ops, i, slot):
        pend = []
        for op in ops:
            if op[0] == "a":
                pend.append((op, attn1(i, slot, op[1], op[2])))
                if len(pend) > _SKEW:
                    o_, st = pend.pop(0)
                    attn2(i, slot, o_[1], o_[2], st)
            else:
                proj(op[0], op[1], 1 - slot)
        for o_, st in pend:
            attn2(i, slot, o_[1], o_[2], st)

    cp_ckv.wait()
    cp_wk(0).wait()
    cp_wv(0).wait()
    for i in range(1, _NP):
        cp_wk(i).start()
        cp_wv(i).start()
        cp_wq(i).start()
    wkb[...] = _unpack_pair(wk_v[0])
    wvb[...] = _unpack_pair(wv_v[0])
    for r in range(_S // _RC):
        proj("k", r, 0)
        proj("v", r, 0)
    cp_x.wait()
    cp_wq(0).wait()
    cp_wo.start()
    cp_wg.start()
    cp_wu.start()
    cp_wd.start()
    wqb[...] = _unpack_pair(wq_v[0])
    for r in range(_S // _RC):
        rs = slice(r * _RC, (r + 1) * _RC)
        xf = _ld(x_v, r * _RC, _RC).astype(_F32)
        mean = jnp.mean(xf, axis=1, keepdims=True)
        d = xf - mean
        var = jnp.mean(d * d, axis=1, keepdims=True)
        _st(ln_v, r * _RC, d * jax.lax.rsqrt(var + _EPS))
        proj("q", r, 0)

    sched = _schedule()

    def pair_body(i, _):
        slot = i % 2
        cp_wq(i + 1).wait()
        cp_wk(i + 1).wait()
        cp_wv(i + 1).wait()
        wkb[...] = _unpack_pair(wk_v[i + 1])
        wvb[...] = _unpack_pair(wv_v[i + 1])
        wqb[...] = _unpack_pair(wq_v[i + 1])
        run_sched(sched, i, slot)
        return 0

    jax.lax.fori_loop(0, _NP - 1, pair_body, 0)
    run_sched([op for op in sched if op[0] == 'a'], _NP - 1, (_NP - 1) % 2)

    cp_wo.wait()
    wr = wr_ref[...].astype(_F32)
    nb = _S // _RB

    def oproj(r, slot):
        acc = None
        for i in range(_NP):
            t = jnp.dot(_ld(ctx_v, r * _RB, _RB, lead=i), _ld(wo_v, i * 256, 256), preferred_element_type=_F32)
            acc = t if acc is None else acc + t
        acc_v[slot] = acc

    def epi(r, slot):
        h = _rb(_ld(x_v, r * _RB, _RB).astype(_F32) + _rb(acc_v[slot]))
        mean = jnp.mean(h, axis=1, keepdims=True)
        d = h - mean
        var = _rb(jnp.mean(d * d, axis=1, keepdims=True))
        ln = _rb(_rb(h - _rb(mean)) / _rb(jnp.sqrt(_rb(var + _EPS))))
        _st(ln_v, r * _RB, ln)
        _st(out_v, r * _RB, h + ln)
        rr = _rb(jnp.sum(ln * wr, axis=1, keepdims=True))
        r_v[r] = jnp.transpose(jnp.broadcast_to(rr, (_RB, 128)))[0:8, :]
        rs = pl.ds(pl.multiple_of(r * (_RB // 2), _RB // 2), _RB // 2)
        pltpu.make_async_copy(out_v.at[rs, :], out_hbm.at[rs, :], sem_o.at[r]).start()

    oproj(0, 0)

    def o_body(r, _):
        oproj(r + 1, (r + 1) % 2)
        epi(r, r % 2)
        return 0

    jax.lax.fori_loop(0, nb - 1, o_body, 0)
    epi(nb - 1, (nb - 1) % 2)

    rrow = jnp.concatenate([r_v[j] for j in range(nb)], axis=1)
    idx = jax.lax.broadcasted_iota(jnp.int32, (8, _S), 1)
    m1 = jnp.max(rrow, axis=1, keepdims=True)
    i1 = jnp.min(jnp.where(rrow == m1, idx, _S), axis=1, keepdims=True)
    rrow2 = jnp.where(idx == i1, -jnp.inf, rrow)
    m2 = jnp.max(rrow2, axis=1, keepdims=True)
    i2 = jnp.min(jnp.where(rrow2 == m2, idx, _S), axis=1, keepdims=True)
    i1s = jnp.clip(jnp.max(i1), 0, _S - 1)
    i2s = jnp.clip(jnp.max(i2), 0, _S - 1)
    g1 = pl.multiple_of((i1s // 16) * 16, 16)
    g2 = pl.multiple_of((i2s // 16) * 16, 16)
    xs = jnp.concatenate([_ld(ln_v, g1, 16), _ld(ln_v, g2, 16)], axis=0)
    cp_wg.wait()
    cp_wu.wait()
    cp_wd.wait()
    g = _rb(jnp.dot(xs, _ld(wg_v, 0, _M), preferred_element_type=_F32))
    u = _rb(jnp.dot(xs, _ld(wu_v, 0, _M), preferred_element_type=_F32))
    g = _rb(g * jax.nn.sigmoid(g))
    y = _rb(jnp.dot((g * u).astype(_BF16), _ld(wd_v, 0, _F), preferred_element_type=_F32))
    rows = jax.lax.broadcasted_iota(jnp.int32, (32, 1), 0)
    grow = jnp.where(rows < 16, rows + g1, rows - 16 + g2)
    rsel = jnp.where(grow == i1s, m1[0:1, :], m2[0:1, :])
    y = _rb(y * _rb(jax.nn.sigmoid(rsel)))
    sel = (grow == i1s) | (grow == i2s)
    upd = jnp.where(sel, _rb(xs.astype(_F32) + y), xs.astype(_F32))
    hbk = _RB // 2
    for r in range(nb):
        pltpu.make_async_copy(out_v.at[r * hbk:(r + 1) * hbk, :], out_hbm.at[r * hbk:(r + 1) * hbk, :], sem_o.at[r]).wait()
    hx = jnp.concatenate([_ld(out_v, g1, 16), _ld(out_v, g2, 16)], axis=0)
    res = (hx.astype(_F32) - xs.astype(_F32) + upd).astype(_BF16)
    _st(out_v, g1, res[0:16])
    _st(out_v, g2, res[16:32])
    for g in (g1, g2):
        rs = pl.ds(pl.multiple_of(g // 2, 8), 8)
        c1 = pltpu.make_async_copy(out_v.at[rs, :], out_hbm.at[rs, :], sem_o.at[0])
        c1.start()
        c1.wait()


@jax.jit
def pallas_sequential_preLN__compressed_kv_cla__moe_arch_mod__prompt_kernel(A_x, A_c_kv, A_w_q, A_w_uk, A_w_uv, A_w_o, B_x, B_w_r, B_w_gate, B_w_up, B_w_down):
    hbm = pl.BlockSpec(memory_space=pl.ANY)
    vm = pltpu.VMEM
    u32 = jnp.uint32
    out = pl.pallas_call(
        _kernel,
        out_shape=jax.ShapeDtypeStruct((_S, _M), _BF16),
        in_specs=[hbm] * 6 + [pl.BlockSpec(memory_space=pltpu.VMEM)] + [hbm] * 3,
        out_specs=hbm,
        scratch_shapes=[
            vm((_S // 2, _M), u32), vm((_S // 2, _DC), u32), vm((_S // 2, _M), u32),
            vm((_NP, _M, _D), u32), vm((_NP, _DC, _D), u32), vm((_NP, _DC, _D), u32),
            vm((_H * _D // 2, _M), u32), vm((_M // 2, _F), u32), vm((_M // 2, _F), u32), vm((_F // 2, _M), u32),
            vm((_M // 2, 2 * _D), u32), vm((_DC // 2, 2 * _D), u32), vm((_DC // 2, 2 * _D), u32),
            vm((2, _S // 2, 2 * _D), u32), vm((2, _S // 2, 2 * _D), u32), vm((2, _S // 2, 2 * _D), u32),
            vm((_NP, _S // 2, 2 * _D), u32), vm((_S // 2, _M), u32), vm((_S // _RB, 8, _RB), _F32),
            vm((2, _RB, _M), _F32),
            pltpu.SemaphoreType.DMA((6,)), pltpu.SemaphoreType.DMA((3, _NP)), pltpu.SemaphoreType.DMA((_S // _RB,)),
        ],
        compiler_params=pltpu.CompilerParams(vmem_limit_bytes=112 * 2**20),
    )(A_x.reshape(_S, _M), A_c_kv.reshape(_S, _DC), A_w_q, A_w_uk, A_w_uv,
      A_w_o.reshape(_H * _D, _M), B_w_r.reshape(1, _M), B_w_gate, B_w_up, B_w_down)
    return out.reshape(1, _S, _M)
```

```python
import os
import numpy as np
import jax
import jax.numpy as jnp
import jax.experimental.pallas as pl
import jax.experimental.pallas.tpu as pltpu

_S, _M, _H, _D, _DC, _F = 2048, 1024, 32, 128, 512, 3584
_NP = _H // 2
_BQ = 256
_EPS = 1e-5
_NT = (((1,), (1,)), ((), ()))
_F32, _BF16 = jnp.float32, jnp.bfloat16
_SCHED = os.environ.get("SCHED", "9")
_DIAG = int(os.environ.get("DIAG", 0))
_RC = int(os.environ.get("RC", 512))
_SKEW = int(os.environ.get("SKEW", 1))
_RB = int(os.environ.get("RB", 256))


def _unpack_pair(w32):
    lo = pltpu.bitcast(w32 << 16, _F32).astype(_BF16)
    hi = pltpu.bitcast(w32 & np.uint32(0xFFFF0000), _F32).astype(_BF16)
    return pltpu.bitcast(jnp.concatenate([lo, hi], axis=1), jnp.uint32)


def _ld(ref, r0, rows, cols=slice(None), lead=None):
    rs = pl.ds(r0 // 2, rows // 2) if isinstance(r0, int) else pl.ds(pl.multiple_of(r0 // 2, rows // 2), rows // 2)
    v = ref[rs, cols] if lead is None else ref[lead, rs, cols]
    return pltpu.bitcast(v, _BF16)


def _st(ref, r0, val, cols=slice(None), lead=None):
    rows = val.shape[0]
    rs = pl.ds(r0 // 2, rows // 2) if isinstance(r0, int) else pl.ds(pl.multiple_of(r0 // 2, rows // 2), rows // 2)
    v = pltpu.bitcast(val.astype(_BF16), jnp.uint32)
    if lead is None:
        ref[rs, cols] = v
    else:
        ref[lead, rs, cols] = v


def _recip(l):
    r = pl.reciprocal(l, approx=True)
    return r + r * (1.0 - l * r)


def _rb(v):
    return v.astype(_BF16).astype(_F32)


def _schedule():
    nq = _S // _BQ
    nr = _S // _RC
    P = [("k", r) for r in range(nr)] + [("v", r) for r in range(nr)] + [("q", r) for r in range(nr)]
    A_seq = [("a", hh, qb) for hh in range(2) for qb in reversed(range(nq))]
    A_int = [("a", hh, qb) for qb in reversed(range(nq)) for hh in range(2)]
    if os.environ.get("POS"):
        pos = [int(t) for t in os.environ["POS"].split(",")]
        A = A_int if os.environ.get("AINT") else A_seq
        if os.environ.get("PORD"):
            P = [P[int(t)] for t in os.environ["PORD"].split(",")]
        out = []
        for j in range(len(A) + 1):
            if j == len(A):
                out.append(("f",))
            out += [p for p, q in zip(P, pos) if q == j]
            if j < len(A):
                out.append(A[j])
        return out
    if _SCHED == "0":
        return P + A_seq
    if _SCHED == "1":
        return P + A_int
    if _SCHED == "2":
        out = []
        slots = len(A_int)
        pos = [int(round(x)) for x in np.linspace(4, slots, len(P))]
        for j, a in enumerate(A_int):
            out.append(a)
            out += [p for p, q in zip(P, pos) if q == j + 1]
        return out
    if _SCHED == "3":
        out = list(A_int[:8])
        rest = A_int[8:]
        for j, a in enumerate(rest):
            out.append(a)
            out += P[(len(P) * j) // len(rest):(len(P) * (j + 1)) // len(rest)]
        return out
    if _SCHED == "4":
        out = P[:len(P) // 2] + A_int[:8]
        rest = A_int[8:]
        P2 = P[len(P) // 2:]
        for j, a in enumerate(rest):
            out.append(a)
            out += P2[(len(P2) * j) // len(rest):(len(P2) * (j + 1)) // len(rest)]
        return out
    if _SCHED == "5":
        A = [("a", hh, qb) for qb in range(nq) for hh in range(2)]
        out = []
        for j, a in enumerate(A):
            out.append(a)
            out += P[(len(P) * j) // len(A):(len(P) * (j + 1)) // len(A)]
        return out
    if _SCHED == "6":
        out = []
        for j, a in enumerate(A_int):
            out.append(a)
            out += P[(len(P) * j) // len(A_int):(len(P) * (j + 1)) // len(A_int)]
        return out
    if _SCHED == "7":
        return A_seq + [("f",)] + P
    if _SCHED == "8":
        return A_int + [("f",)] + P
    if _SCHED == "9":
        return A_seq[:7] + P[:6] + A_seq[7:] + [("f",)] + P[6:]
    if _SCHED == "10":
        return A_seq[:-2] + P[:4] + A_seq[-2:] + [("f",)] + P[4:]
    if _SCHED == "11":
        return A_seq[:-4] + P[:4] + A_seq[-4:-2] + P[4:8] + A_seq[-2:] + [("f",)] + P[8:]
    if _SCHED == "12":
        return A_seq[:6] + P[:4] + A_seq[6:-2] + P[4:8] + A_seq[-2:] + [("f",)] + P[8:]
    raise ValueError


def _kernel(x_hbm, ckv_hbm, wq_hbm, wk_hbm, wv_hbm, wo_hbm, wr_ref, wg_hbm, wu_hbm, wd_hbm,
            out_hbm,
            x_v, ckv_v, ln_v, wq_v, wk_v, wv_v, wo_v, wg_v, wu_v, wd_v,
            wqb, wkb, wvb, q_v, k_v, v_v, ctx_v, out_v, r_v, acc_v, rr_v,
            sem_a, sem_w, sem_o, sem_x):
    wq32 = wq_hbm.bitcast(jnp.uint32)
    wk32 = wk_hbm.bitcast(jnp.uint32)
    wv32 = wv_hbm.bitcast(jnp.uint32)
    x_hbm, ckv_hbm, wo_hbm, wg_hbm, wu_hbm, wd_hbm, out_hbm = [
        t.bitcast(jnp.uint32) for t in (x_hbm, ckv_hbm, wo_hbm, wg_hbm, wu_hbm, wd_hbm, out_hbm)]

    cp_ckv = pltpu.make_async_copy(ckv_hbm, ckv_v, sem_a.at[0])
    _XC = 256
    nxc = _S // _XC

    def cp_x(c):
        return pltpu.make_async_copy(x_hbm.at[c * _XC // 2:(c + 1) * _XC // 2], x_v.at[c * _XC // 2:(c + 1) * _XC // 2], sem_x.at[c])

    cp_wo = pltpu.make_async_copy(wo_hbm, wo_v, sem_a.at[2])
    cp_wg = pltpu.make_async_copy(wg_hbm, wg_v, sem_a.at[3])
    cp_wu = pltpu.make_async_copy(wu_hbm, wu_v, sem_a.at[4])
    cp_wd = pltpu.make_async_copy(wd_hbm, wd_v, sem_a.at[5])

    def cp_wq(i):
        return pltpu.make_async_copy(wq32.at[:, i, :], wq_v.at[i], sem_w.at[0, i])

    def cp_wk(i):
        return pltpu.make_async_copy(wk32.at[:, i, :], wk_v.at[i], sem_w.at[1, i])

    def cp_wv(i):
        return pltpu.make_async_copy(wv32.at[:, i, :], wv_v.at[i], sem_w.at[2, i])

    qscale = np.float32(_D ** -0.5 * np.log2(np.e))

    def proj(kind, r, slot):
        r0 = r * _RC
        if kind == "k":
            _st(k_v, r0, jnp.dot(_ld(ckv_v, r0, _RC), _ld(wkb, 0, _DC), preferred_element_type=_F32), lead=slot)
        elif kind == "v":
            _st(v_v, r0, jnp.dot(_ld(ckv_v, r0, _RC), _ld(wvb, 0, _DC), preferred_element_type=_F32), lead=slot)
        else:
            q = jnp.dot(_ld(ln_v, r0, _RC), _ld(wqb, 0, _M), preferred_element_type=_F32)
            _st(q_v, r0, q * qscale, lead=slot)

    hb = _BQ // 2

    def attn1(i, slot, hh, qb):
        hs = slice(hh * _D, (hh + 1) * _D)
        q = _ld(q_v, qb * _BQ, _BQ, hs, slot)
        ri = jax.lax.broadcasted_iota(jnp.int32, (hb, hb), 0)
        ci = jax.lax.broadcasted_iota(jnp.int32, (hb, hb), 1)
        keep = ci <= ri
        n = qb * _BQ + hb
        s1 = jax.lax.dot_general(q, _ld(k_v, 0, n, hs, slot), _NT, preferred_element_type=_F32)
        s2 = jax.lax.dot_general(q[hb:], _ld(k_v, n, hb, hs, slot), _NT, preferred_element_type=_F32)
        su = jnp.where(keep, s1[:hb, n - hb:], -1e9)
        if qb > 0:
            su = jnp.concatenate([s1[:hb, :n - hb], su], axis=1)
        sl = jnp.concatenate([s1[hb:], jnp.where(keep, s2, -1e9)], axis=1)
        return su, sl, jnp.max(su, axis=1, keepdims=True), jnp.max(sl, axis=1, keepdims=True)

    def attn2(i, slot, hh, qb, st):
        hs = slice(hh * _D, (hh + 1) * _D)
        su, sl, mu, ml = st
        n = qb * _BQ + hb
        pu = jnp.exp2(su - mu)
        pl_ = jnp.exp2(sl - ml)
        lu = jnp.sum(pu, axis=1, keepdims=True)
        ll = jnp.sum(pl_, axis=1, keepdims=True)
        p1 = jnp.concatenate([pu, pl_[:, :n]], axis=0).astype(_BF16)
        o = jnp.dot(p1, _ld(v_v, 0, n, hs, slot), preferred_element_type=_F32)
        o2 = jnp.dot(pl_[:, n:].astype(_BF16), _ld(v_v, n, hb, hs, slot), preferred_element_type=_F32)
        _st(ctx_v, qb * _BQ, o[:hb] * _recip(lu), hs, i)
        _st(ctx_v, qb * _BQ + hb, (o[hb:] + o2) * _recip(ll), hs, i)

    def run_sched(ops, i, slot):
        pend = []
        for op in ops:
            if op[0] == "a":
                pend.append((op, attn1(i, slot, op[1], op[2])))
                if len(pend) > _SKEW:
                    o_, st = pend.pop(0)
                    attn2(i, slot, o_[1], o_[2], st)
            elif op[0] == "f":
                for o_, st in pend:
                    attn2(i, slot, o_[1], o_[2], st)
                pend = []
            else:
                proj(op[0], op[1], 1 - slot)
        for o_, st in pend:
            attn2(i, slot, o_[1], o_[2], st)

    early = [cp_x(0), cp_wq(0)] + [cp_x(c) for c in range(1, nxc)] + [cp_ckv, cp_wk(0), cp_wv(0)]
    LOOK = int(os.environ.get("LOOK", 3))
    state = {"started": 0}

    def advance(n):
        while state["started"] < min(n, len(early)):
            early[state["started"]].start()
            state["started"] += 1

    def wait_early(j):
        advance(j + LOOK)
        early[j].wait()

    def ln1(c):
        xf = _ld(x_v, c * _XC, _XC).astype(_F32)
        mean = jnp.mean(xf, axis=1, keepdims=True)
        d = xf - mean
        var = jnp.mean(d * d, axis=1, keepdims=True)
        _st(ln_v, c * _XC, d * jax.lax.rsqrt(var + _EPS))

    wait_early(0)
    ln1(0)
    wait_early(1)
    for c in range(nxc):
        if c + 1 < nxc:
            wait_early(c + 2)
        if c == 0:
            wqb[...] = _unpack_pair(wq_v[0])
        q = jnp.dot(_ld(ln_v, c * _XC, _XC), _ld(wqb, 0, _M), preferred_element_type=_F32)
        _st(q_v, c * _XC, q * qscale, lead=0)
        if c + 1 < nxc:
            ln1(c + 1)
    advance(len(early))
    cp_ckv.wait()
    cp_wk(0).wait()
    cp_wv(0).wait()
    for i in range(1, _NP):
        cp_wk(i).start()
        cp_wv(i).start()
        cp_wq(i).start()
    cp_wo.start()
    cp_wg.start()
    cp_wu.start()
    cp_wd.start()
    wkb[...] = _unpack_pair(wk_v[0])
    wvb[...] = _unpack_pair(wv_v[0])
    for r in range(_S // _RC):
        proj("k", r, 0)
        proj("v", r, 0)

    sched = _schedule()

    def pair_body(i, _):
        slot = i % 2
        cp_wq(i + 1).wait()
        cp_wk(i + 1).wait()
        cp_wv(i + 1).wait()
        wkb[...] = _unpack_pair(wk_v[i + 1])
        wvb[...] = _unpack_pair(wv_v[i + 1])
        wqb[...] = _unpack_pair(wq_v[i + 1])
        run_sched(sched, i, slot)
        return 0

    jax.lax.fori_loop(0, _NP - 1, pair_body, 0)
    run_sched([op for op in sched if op[0] == 'a'], _NP - 1, (_NP - 1) % 2)

    cp_wo.wait()
    wr = wr_ref[...].astype(_F32)
    nb = _S // _RB

    _EC = int(os.environ.get("EC", 4))

    def oproj(r, slot, inter=None):
        if int(os.environ.get("ONE", 0)):
            lhs = jnp.concatenate([_ld(ctx_v, r * _RB, _RB, lead=i) for i in range(_NP)], axis=1)
            NS = int(os.environ.get("ONE"))
            for j in range(NS):
                cs = slice(j * _M // NS, (j + 1) * _M // NS)
                if inter is not None and j < _EC:
                    inter(j)
                acc_v[slot, :, cs] = jnp.dot(lhs, _ld(wo_v, 0, _H * _D, cs), preferred_element_type=_F32)
            return
        acc = None
        for i in range(_NP):
            t = jnp.dot(_ld(ctx_v, r * _RB, _RB, lead=i), _ld(wo_v, i * 256, 256), preferred_element_type=_F32)
            acc = t if acc is None else acc + t
            if inter is not None and (i + 1) % (_NP // _EC) == (_NP // _EC) // 2:
                inter(i // (_NP // _EC))
        acc_v[slot] = acc

    def epi(r, slot, c, nc):
        cr = _RB // nc
        r0 = r * _RB + c * cr
        h = _rb(_ld(x_v, r0, cr).astype(_F32) + acc_v[slot, c * cr:(c + 1) * cr, :])
        mean = jnp.mean(h, axis=1, keepdims=True)
        d = h - mean
        var = _rb(jnp.mean(d * d, axis=1, keepdims=True))
        rs_ = 1.0 / _rb(jnp.sqrt(_rb(var + _EPS)))
        ln = _rb(d * rs_)
        _st(ln_v, r0, ln)
        _st(x_v, r0, h)
        _st(out_v, r0, h + ln)
        rr_v[c * cr:(c + 1) * cr, :] = jnp.broadcast_to(_rb(jnp.sum(ln * wr, axis=1, keepdims=True)), (cr, 128))

    def fin(r):
        r_v[r] = jnp.transpose(rr_v[...])[0:8, :]
        put(r)

    def put(r):
        rs = pl.ds(pl.multiple_of(r * (_RB // 2), _RB // 2), _RB // 2)
        pltpu.make_async_copy(out_v.at[rs, :], out_hbm.at[rs, :], sem_o.at[r]).start()

    acc_v[1] = jnp.zeros((_RB, _M), _F32)

    def o_body(j, _):
        r = jnp.maximum(j - 1, 0)
        oproj(j, j % 2, lambda c: epi(r, 1 - j % 2, c, _EC))
        r_v[r] = jnp.transpose(rr_v[...])[0:8, :]

        @pl.when(j > 0)
        def _():
            put(r)
        return 0

    jax.lax.fori_loop(0, nb, o_body, 0)
    epi(nb - 1, (nb - 1) % 2, 0, 1)
    fin(nb - 1)

    rrow = jnp.concatenate([r_v[j] for j in range(nb)], axis=1)
    idx = jax.lax.broadcasted_iota(jnp.int32, (8, _S), 1)
    m1 = jnp.max(rrow, axis=1, keepdims=True)
    i1 = jnp.min(jnp.where(rrow == m1, idx, _S), axis=1, keepdims=True)
    rrow2 = jnp.where(idx == i1, -jnp.inf, rrow)
    m2 = jnp.max(rrow2, axis=1, keepdims=True)
    i2 = jnp.min(jnp.where(rrow2 == m2, idx, _S), axis=1, keepdims=True)
    i1s = jnp.clip(jnp.max(i1), 0, _S - 1)
    i2s = jnp.clip(jnp.max(i2), 0, _S - 1)
    def row_f32(ref, i):
        w = ref[pl.ds(i // 2, 1), :]
        return pltpu.bitcast(jnp.where(i % 2 == 0, w << 16, w & np.uint32(0xFFFF0000)), _F32)

    rows = jax.lax.broadcasted_iota(jnp.int32, (16, 1), 0)

    def two_rows(ref):
        return jnp.where(rows == 0, row_f32(ref, i1s), jnp.where(rows == 1, row_f32(ref, i2s), 0.0))

    xs = two_rows(ln_v)
    hs_ = two_rows(x_v)
    xb = xs.astype(_BF16)
    cp_wg.wait()
    cp_wu.wait()
    cp_wd.wait()
    g = _rb(jnp.dot(xb, _ld(wg_v, 0, _M), preferred_element_type=_F32))
    u = _rb(jnp.dot(xb, _ld(wu_v, 0, _M), preferred_element_type=_F32))
    g = _rb(g * jax.nn.sigmoid(g))
    y = _rb(jnp.dot((g * u).astype(_BF16), _ld(wd_v, 0, _F), preferred_element_type=_F32))
    rsel = jnp.where(rows == 0, m1[0:1, :], m2[0:1, :])
    y = _rb(y * _rb(jax.nn.sigmoid(rsel)))
    res = hs_ + _rb(xs + y)
    hbk = _RB // 2
    for r in range(nb):
        pltpu.make_async_copy(out_v.at[r * hbk:(r + 1) * hbk, :], out_hbm.at[r * hbk:(r + 1) * hbk, :], sem_o.at[r]).wait()

    def patch(g, sem):
        grow = rows + g
        cur = _ld(out_v, g, 16).astype(_F32)
        new = jnp.where(grow == i1s, res[0:1], jnp.where(grow == i2s, res[1:2], cur))
        _st(out_v, g, new)
        rs = pl.ds(pl.multiple_of(g // 2, 8), 8)
        return pltpu.make_async_copy(out_v.at[rs, :], out_hbm.at[rs, :], sem)

    g1 = pl.multiple_of((i1s // 16) * 16, 16)
    g2 = pl.multiple_of((i2s // 16) * 16, 16)
    c1 = patch(g1, sem_o.at[0])
    c1.start()

    @pl.when(g2 != g1)
    def _():
        c2 = patch(g2, sem_o.at[1])
        c2.start()
        c2.wait()

    c1.wait()


@jax.jit
def pallas_sequential_preLN__compressed_kv_cla__moe_arch_mod__prompt_kernel(A_x, A_c_kv, A_w_q, A_w_uk, A_w_uv, A_w_o, B_x, B_w_r, B_w_gate, B_w_up, B_w_down):
    hbm = pl.BlockSpec(memory_space=pl.ANY)
    vm = pltpu.VMEM
    u32 = jnp.uint32
    out = pl.pallas_call(
        _kernel,
        out_shape=jax.ShapeDtypeStruct((_S, _M), _BF16),
        in_specs=[hbm] * 6 + [pl.BlockSpec(memory_space=pltpu.VMEM)] + [hbm] * 3,
        out_specs=hbm,
        scratch_shapes=[
            vm((_S // 2, _M), u32), vm((_S // 2, _DC), u32), vm((_S // 2, _M), u32),
            vm((_NP, _M, _D), u32), vm((_NP, _DC, _D), u32), vm((_NP, _DC, _D), u32),
            vm((_H * _D // 2, _M), u32), vm((_M // 2, _F), u32), vm((_M // 2, _F), u32), vm((_F // 2, _M), u32),
            vm((_M // 2, 2 * _D), u32), vm((_DC // 2, 2 * _D), u32), vm((_DC // 2, 2 * _D), u32),
            vm((2, _S // 2, 2 * _D), u32), vm((2, _S // 2, 2 * _D), u32), vm((2, _S // 2, 2 * _D), u32),
            vm((_NP, _S // 2, 2 * _D), u32), vm((_S // 2, _M), u32), vm((_S // _RB, 8, _RB), _F32),
            vm((2, _RB, _M), _F32), vm((_RB, 128), _F32),
            pltpu.SemaphoreType.DMA((6,)), pltpu.SemaphoreType.DMA((3, _NP)), pltpu.SemaphoreType.DMA((_S // _RB,)), pltpu.SemaphoreType.DMA((8,)),
        ],
        compiler_params=pltpu.CompilerParams(vmem_limit_bytes=120 * 2**20, flags={'XLA_TPU_EVENLY_DISTRIBUTE_CRITICAL_NODES': True}),
    )(A_x.reshape(_S, _M), A_c_kv.reshape(_S, _DC), A_w_q, A_w_uk, A_w_uv,
      A_w_o.reshape(_H * _D, _M), B_w_r.reshape(1, _M), B_w_gate, B_w_up, B_w_down)
    return out.reshape(1, _S, _M)
```

```python
import os
import numpy as np
import jax
import jax.numpy as jnp
import jax.experimental.pallas as pl
import jax.experimental.pallas.tpu as pltpu

_S, _M, _H, _D, _DC, _F = 2048, 1024, 32, 128, 512, 3584
_NP = _H // 2
_BQ = 256
_EPS = 1e-5
_NT = (((1,), (1,)), ((), ()))
_F32, _BF16 = jnp.float32, jnp.bfloat16
_SCHED = os.environ.get("SCHED", "9")
_DIAG = int(os.environ.get("DIAG", 0))
_RC = int(os.environ.get("RC", 512))
_SKEW = int(os.environ.get("SKEW", 3))
_RB = int(os.environ.get("RB", 256))


def _unpack_pair(w32):
    lo = pltpu.bitcast(w32 << 16, _F32).astype(_BF16)
    hi = pltpu.bitcast(w32 & np.uint32(0xFFFF0000), _F32).astype(_BF16)
    return pltpu.bitcast(jnp.concatenate([lo, hi], axis=1), jnp.uint32)


def _ld(ref, r0, rows, cols=slice(None), lead=None):
    rs = pl.ds(r0 // 2, rows // 2) if isinstance(r0, int) else pl.ds(pl.multiple_of(r0 // 2, rows // 2), rows // 2)
    v = ref[rs, cols] if lead is None else ref[lead, rs, cols]
    return pltpu.bitcast(v, _BF16)


def _st(ref, r0, val, cols=slice(None), lead=None):
    rows = val.shape[0]
    rs = pl.ds(r0 // 2, rows // 2) if isinstance(r0, int) else pl.ds(pl.multiple_of(r0 // 2, rows // 2), rows // 2)
    v = pltpu.bitcast(val.astype(_BF16), jnp.uint32)
    if lead is None:
        ref[rs, cols] = v
    else:
        ref[lead, rs, cols] = v


def _recip(l):
    r = pl.reciprocal(l, approx=True)
    return r + r * (1.0 - l * r)


def _rb(v):
    return v.astype(_BF16).astype(_F32)


def _schedule():
    nq = _S // _BQ * (2 if int(os.environ.get('Q128', 1)) else 1)
    nr = _S // _RC
    P = [("k", r) for r in range(nr)] + [("v", r) for r in range(nr)] + [("q", r) for r in range(nr)]
    A_seq = [("a", hh, qb) for hh in range(2) for qb in reversed(range(nq))]
    A_int = [("a", hh, qb) for qb in reversed(range(nq)) for hh in range(2)]
    if os.environ.get("POS"):
        pos = [int(t) for t in os.environ["POS"].split(",")]
        A = A_int if os.environ.get("AINT") else A_seq
        if os.environ.get("PORD"):
            P = [P[int(t)] for t in os.environ["PORD"].split(",")]
        out = []
        for j in range(len(A) + 1):
            if j == len(A):
                out.append(("f",))
            out += [p for p, q in zip(P, pos) if q == j]
            if j < len(A):
                out.append(A[j])
        return out
    if _SCHED == "0":
        return P + A_seq
    if _SCHED == "1":
        return P + A_int
    if _SCHED == "2":
        out = []
        slots = len(A_int)
        pos = [int(round(x)) for x in np.linspace(4, slots, len(P))]
        for j, a in enumerate(A_int):
            out.append(a)
            out += [p for p, q in zip(P, pos) if q == j + 1]
        return out
    if _SCHED == "3":
        out = list(A_int[:8])
        rest = A_int[8:]
        for j, a in enumerate(rest):
            out.append(a)
            out += P[(len(P) * j) // len(rest):(len(P) * (j + 1)) // len(rest)]
        return out
    if _SCHED == "4":
        out = P[:len(P) // 2] + A_int[:8]
        rest = A_int[8:]
        P2 = P[len(P) // 2:]
        for j, a in enumerate(rest):
            out.append(a)
            out += P2[(len(P2) * j) // len(rest):(len(P2) * (j + 1)) // len(rest)]
        return out
    if _SCHED == "5":
        A = [("a", hh, qb) for qb in range(nq) for hh in range(2)]
        out = []
        for j, a in enumerate(A):
            out.append(a)
            out += P[(len(P) * j) // len(A):(len(P) * (j + 1)) // len(A)]
        return out
    if _SCHED == "6":
        out = []
        for j, a in enumerate(A_int):
            out.append(a)
            out += P[(len(P) * j) // len(A_int):(len(P) * (j + 1)) // len(A_int)]
        return out
    if _SCHED == "7":
        return A_seq + [("f",)] + P
    if _SCHED == "8":
        return A_int + [("f",)] + P
    if _SCHED == "9":
        return A_seq[:nq - 1] + P[:len(P) // 2] + A_seq[nq - 1:] + [("f",)] + P[len(P) // 2:]
    if _SCHED == "10":
        return A_seq[:-2] + P[:4] + A_seq[-2:] + [("f",)] + P[4:]
    if _SCHED == "11":
        return A_seq[:-4] + P[:4] + A_seq[-4:-2] + P[4:8] + A_seq[-2:] + [("f",)] + P[8:]
    if _SCHED == "12":
        return A_seq[:6] + P[:4] + A_seq[6:-2] + P[4:8] + A_seq[-2:] + [("f",)] + P[8:]
    raise ValueError


def _kernel(x_hbm, ckv_hbm, wq_hbm, wk_hbm, wv_hbm, wo_hbm, wr_ref, wg_hbm, wu_hbm, wd_hbm,
            out_hbm,
            x_v, ckv_v, ln_v, wq_v, wk_v, wv_v, wo_v, wg_v, wu_v, wd_v,
            wqb, wkb, wvb, q_v, k_v, v_v, ctx_v, out_v, r_v, acc_v, rr_v,
            sem_a, sem_w, sem_o, sem_x, sem_k):
    wq32 = wq_hbm.bitcast(jnp.uint32)
    wk32 = wk_hbm.bitcast(jnp.uint32)
    wv32 = wv_hbm.bitcast(jnp.uint32)
    x_hbm, ckv_hbm, wo_hbm, wg_hbm, wu_hbm, wd_hbm, out_hbm = [
        t.bitcast(jnp.uint32) for t in (x_hbm, ckv_hbm, wo_hbm, wg_hbm, wu_hbm, wd_hbm, out_hbm)]

    nkc = _S // _RC

    def cp_ck(c):
        return pltpu.make_async_copy(ckv_hbm.at[rows_u32(c, _RC)], ckv_v.at[rows_u32(c, _RC)], sem_k.at[c])

    _XC = 256
    nxc = _S // _XC

    def rows_u32(c, n):
        if isinstance(c, int):
            return pl.ds(c * (n // 2), n // 2)
        return pl.ds(pl.multiple_of(c * (n // 2), n // 2), n // 2)

    def cp_x(c):
        return pltpu.make_async_copy(x_hbm.at[rows_u32(c, _XC)], x_v.at[rows_u32(c, _XC)], sem_x.at[c])

    cp_wo = pltpu.make_async_copy(wo_hbm, wo_v, sem_a.at[2])
    cp_wg = pltpu.make_async_copy(wg_hbm, wg_v, sem_a.at[3])
    cp_wu = pltpu.make_async_copy(wu_hbm, wu_v, sem_a.at[4])
    cp_wd = pltpu.make_async_copy(wd_hbm, wd_v, sem_a.at[5])

    def cp_wq(i):
        return pltpu.make_async_copy(wq32.at[:, i, :], wq_v.at[i], sem_w.at[0, i])

    def cp_wk(i):
        return pltpu.make_async_copy(wk32.at[:, i, :], wk_v.at[i], sem_w.at[1, i])

    def cp_wv(i):
        return pltpu.make_async_copy(wv32.at[:, i, :], wv_v.at[i], sem_w.at[2, i])

    qscale = np.float32(_D ** -0.5 * np.log2(np.e))

    def proj(kind, r, slot):
        r0 = r * _RC
        if kind == "k":
            _st(k_v, r0, jnp.dot(_ld(ckv_v, r0, _RC), _ld(wkb, 0, _DC), preferred_element_type=_F32), lead=slot)
        elif kind == "v":
            _st(v_v, r0, jnp.dot(_ld(ckv_v, r0, _RC), _ld(wvb, 0, _DC), preferred_element_type=_F32), lead=slot)
        else:
            q = jnp.dot(_ld(ln_v, r0, _RC), _ld(wqb, 0, _M), preferred_element_type=_F32)
            _st(q_v, r0, q * qscale, lead=slot)

    hb = _BQ // 2

    def attn1(i, slot, hh, qb):
        hs = slice(hh * _D, (hh + 1) * _D)
        q = _ld(q_v, qb * _BQ, _BQ, hs, slot)
        ri = jax.lax.broadcasted_iota(jnp.int32, (hb, hb), 0)
        ci = jax.lax.broadcasted_iota(jnp.int32, (hb, hb), 1)
        keep = ci <= ri
        n = qb * _BQ + hb
        s1 = jax.lax.dot_general(q, _ld(k_v, 0, n, hs, slot), _NT, preferred_element_type=_F32)
        s2 = jax.lax.dot_general(q[hb:], _ld(k_v, n, hb, hs, slot), _NT, preferred_element_type=_F32)
        su = jnp.where(keep, s1[:hb, n - hb:], -1e9)
        if qb > 0:
            su = jnp.concatenate([s1[:hb, :n - hb], su], axis=1)
        sl = jnp.concatenate([s1[hb:], jnp.where(keep, s2, -1e9)], axis=1)
        return su, sl, jnp.max(su, axis=1, keepdims=True), jnp.max(sl, axis=1, keepdims=True)

    def attn2(i, slot, hh, qb, st):
        hs = slice(hh * _D, (hh + 1) * _D)
        su, sl, mu, ml = st
        n = qb * _BQ + hb
        pu = jnp.exp2(su - mu)
        pl_ = jnp.exp2(sl - ml)
        if int(os.environ.get("PB", 1)):
            pu = pu.astype(_BF16)
            pl_ = pl_.astype(_BF16)
        lu = jnp.sum(pu.astype(_F32), axis=1, keepdims=True)
        ll = jnp.sum(pl_.astype(_F32), axis=1, keepdims=True)
        if int(os.environ.get("PVS", 1)):
            ou = jnp.dot(pu.astype(_BF16), _ld(v_v, 0, n, hs, slot), preferred_element_type=_F32)
            ol = jnp.dot(pl_.astype(_BF16), _ld(v_v, 0, n + hb, hs, slot), preferred_element_type=_F32)
            _st(ctx_v, qb * _BQ, ou * _recip(lu), hs, i)
            _st(ctx_v, qb * _BQ + hb, ol * _recip(ll), hs, i)
            return
        p1 = jnp.concatenate([pu, pl_[:, :n]], axis=0).astype(_BF16)
        o = jnp.dot(p1, _ld(v_v, 0, n, hs, slot), preferred_element_type=_F32)
        o2 = jnp.dot(pl_[:, n:].astype(_BF16), _ld(v_v, n, hb, hs, slot), preferred_element_type=_F32)
        _st(ctx_v, qb * _BQ, o[:hb] * _recip(lu), hs, i)
        _st(ctx_v, qb * _BQ + hb, (o[hb:] + o2) * _recip(ll), hs, i)

    def attn1h(i, slot, hh, qb):
        hs = slice(hh * _D, (hh + 1) * _D)
        q = _ld(q_v, qb * hb, hb, hs, slot)
        ri = jax.lax.broadcasted_iota(jnp.int32, (hb, hb), 0)
        ci = jax.lax.broadcasted_iota(jnp.int32, (hb, hb), 1)
        n = (qb + 1) * hb
        s1 = jax.lax.dot_general(q, _ld(k_v, 0, n, hs, slot), _NT, preferred_element_type=_F32)
        sd = jnp.where(ci <= ri, s1[:, n - hb:], -1e9)
        if qb > 0:
            sd = jnp.concatenate([s1[:, :n - hb], sd], axis=1)
        return sd, jnp.max(sd, axis=1, keepdims=True)

    def attn2h(i, slot, hh, qb, st):
        hs = slice(hh * _D, (hh + 1) * _D)
        sd, m = st
        n = (qb + 1) * hb
        p = jnp.exp2(sd - m)
        if int(os.environ.get("PB", 1)):
            p = p.astype(_BF16)
        l = jnp.sum(p.astype(_F32), axis=1, keepdims=True)
        o = jnp.dot(p.astype(_BF16), _ld(v_v, 0, n, hs, slot), preferred_element_type=_F32)
        _st(ctx_v, qb * hb, o * _recip(l), hs, i)

    if int(os.environ.get("Q128", 1)):
        attn1, attn2 = attn1h, attn2h

    def run_sched(ops, i, slot):
        pend = []
        for op in ops:
            if op[0] == "a":
                pend.append((op, attn1(i, slot, op[1], op[2])))
                if len(pend) > _SKEW:
                    o_, st = pend.pop(0)
                    attn2(i, slot, o_[1], o_[2], st)
            elif op[0] == "f":
                for o_, st in pend:
                    attn2(i, slot, o_[1], o_[2], st)
                pend = []
            else:
                proj(op[0], op[1], 1 - slot)
        for o_, st in pend:
            attn2(i, slot, o_[1], o_[2], st)

    early = [cp_wk(0), cp_wv(0)] + [cp_ck(c) for c in range(nkc)] + [cp_wq(0)] + [cp_x(c) for c in range(nxc)]
    for cp in early:
        cp.start()

    def ln1(c):
        xf = _ld(x_v, c * _XC, _XC).astype(_F32)
        mean = jnp.mean(xf, axis=1, keepdims=True)
        d = xf - mean
        var = jnp.mean(d * d, axis=1, keepdims=True)
        _st(ln_v, c * _XC, d * jax.lax.rsqrt(var + _EPS))

    cp_wk(0).wait()
    cp_wv(0).wait()
    wkb[...] = _unpack_pair(wk_v[0])
    wvb[...] = _unpack_pair(wv_v[0])

    def kv_body(c, _):
        cp_ck(c).wait()
        proj("k", c, 0)
        proj("v", c, 0)
        return 0

    jax.lax.fori_loop(0, nkc - 1, kv_body, 0)
    cp_ck(nkc - 1).wait()
    cp_wq(0).wait()
    cp_x(0).wait()
    proj("k", nkc - 1, 0)
    proj("v", nkc - 1, 0)
    wqb[...] = _unpack_pair(wq_v[0])
    ln1(0)

    def q0(c):
        q = jnp.dot(_ld(ln_v, c * _XC, _XC), _ld(wqb, 0, _M), preferred_element_type=_F32)
        _st(q_v, c * _XC, q * qscale, lead=0)

    def q_body(c, _):
        cp_x(c + 1).wait()
        q0(c)
        ln1(c + 1)
        return 0

    jax.lax.fori_loop(0, nxc - 1, q_body, 0)
    cp_wk(1).start()
    cp_wv(1).start()
    cp_wq(1).start()
    q0(nxc - 1)

    sched = _schedule()

    def pair_body(i, _):
        slot = i % 2

        @pl.when(i == 0)
        def _():
            for t in range(2, _NP):
                cp_wk(t).start()
                cp_wv(t).start()
                cp_wq(t).start()
            cp_wo.start()
            cp_wg.start()
            cp_wu.start()
            cp_wd.start()

        cp_wq(i + 1).wait()
        cp_wk(i + 1).wait()
        cp_wv(i + 1).wait()
        wkb[...] = _unpack_pair(wk_v[i + 1])
        wvb[...] = _unpack_pair(wv_v[i + 1])
        wqb[...] = _unpack_pair(wq_v[i + 1])
        run_sched(sched, i, slot)
        return 0

    jax.lax.fori_loop(0, _NP - 1, pair_body, 0)
    run_sched([op for op in sched if op[0] == 'a'], _NP - 1, (_NP - 1) % 2)

    cp_wo.wait()
    wr = wr_ref[...].astype(_F32)
    nb = _S // _RB

    _EC = int(os.environ.get("EC", 4))

    def oproj(r, slot, inter=None):
        if int(os.environ.get("ONE", 0)):
            lhs = jnp.concatenate([_ld(ctx_v, r * _RB, _RB, lead=i) for i in range(_NP)], axis=1)
            NS = int(os.environ.get("ONE"))
            for j in range(NS):
                cs = slice(j * _M // NS, (j + 1) * _M // NS)
                if inter is not None and j < _EC:
                    inter(j)
                acc_v[slot, :, cs] = jnp.dot(lhs, _ld(wo_v, 0, _H * _D, cs), preferred_element_type=_F32)
            return
        acc = None
        for i in range(_NP):
            t = jnp.dot(_ld(ctx_v, r * _RB, _RB, lead=i), _ld(wo_v, i * 256, 256), preferred_element_type=_F32)
            acc = t if acc is None else acc + t
            if inter is not None and (i + 1) % (_NP // _EC) == (_NP // _EC) // 2:
                inter(i // (_NP // _EC))
        acc_v[slot] = acc

    def epi(r, slot, c, nc):
        cr = _RB // nc
        r0 = r * _RB + c * cr
        h = _rb(_ld(x_v, r0, cr).astype(_F32) + acc_v[slot, c * cr:(c + 1) * cr, :])
        mean = jnp.mean(h, axis=1, keepdims=True)
        d = h - mean
        var = _rb(jnp.mean(d * d, axis=1, keepdims=True))
        rs_ = 1.0 / _rb(jnp.sqrt(_rb(var + _EPS)))
        ln = _rb(d * rs_)
        _st(ln_v, r0, ln)
        _st(x_v, r0, h)
        _st(out_v, r0, h + ln)
        rr_v[c * cr:(c + 1) * cr, :] = jnp.broadcast_to(_rb(jnp.sum(ln * wr, axis=1, keepdims=True)), (cr, 128))

    def fin(r):
        r_v[r] = jnp.transpose(rr_v[...])[0:8, :]
        put(r)

    def put(r):
        rs = pl.ds(pl.multiple_of(r * (_RB // 2), _RB // 2), _RB // 2)
        pltpu.make_async_copy(out_v.at[rs, :], out_hbm.at[rs, :], sem_o.at[r]).start()

    acc_v[1] = jnp.zeros((_RB, _M), _F32)

    def o_body(j, _):
        r = jnp.maximum(j - 1, 0)
        oproj(j, j % 2, lambda c: epi(r, 1 - j % 2, c, _EC))
        r_v[r] = jnp.transpose(rr_v[...])[0:8, :]

        @pl.when(j > 0)
        def _():
            put(r)
        return 0

    jax.lax.fori_loop(0, nb, o_body, 0)
    epi(nb - 1, (nb - 1) % 2, 0, 1)
    fin(nb - 1)

    rrow = jnp.concatenate([r_v[j] for j in range(nb)], axis=1)
    idx = jax.lax.broadcasted_iota(jnp.int32, (8, _S), 1)
    m1 = jnp.max(rrow, axis=1, keepdims=True)
    i1 = jnp.min(jnp.where(rrow == m1, idx, _S), axis=1, keepdims=True)
    rrow2 = jnp.where(idx == i1, -jnp.inf, rrow)
    m2 = jnp.max(rrow2, axis=1, keepdims=True)
    i2 = jnp.min(jnp.where(rrow2 == m2, idx, _S), axis=1, keepdims=True)
    i1s = jnp.clip(jnp.max(i1), 0, _S - 1)
    i2s = jnp.clip(jnp.max(i2), 0, _S - 1)
    def row_f32(ref, i):
        w = ref[pl.ds(i // 2, 1), :]
        return pltpu.bitcast(jnp.where(i % 2 == 0, w << 16, w & np.uint32(0xFFFF0000)), _F32)

    rows = jax.lax.broadcasted_iota(jnp.int32, (16, 1), 0)

    def two_rows(ref):
        return jnp.where(rows == 0, row_f32(ref, i1s), jnp.where(rows == 1, row_f32(ref, i2s), 0.0))

    xs = two_rows(ln_v)
    hs_ = two_rows(x_v)
    xb = xs.astype(_BF16)
    cp_wg.wait()
    cp_wu.wait()
    cp_wd.wait()
    g = _rb(jnp.dot(xb, _ld(wg_v, 0, _M), preferred_element_type=_F32))
    u = _rb(jnp.dot(xb, _ld(wu_v, 0, _M), preferred_element_type=_F32))
    g = _rb(g * jax.nn.sigmoid(g))
    y = _rb(jnp.dot((g * u).astype(_BF16), _ld(wd_v, 0, _F), preferred_element_type=_F32))
    rsel = jnp.where(rows == 0, m1[0:1, :], m2[0:1, :])
    y = _rb(y * _rb(jax.nn.sigmoid(rsel)))
    res = hs_ + _rb(xs + y)
    hbk = _RB // 2
    for r in range(nb):
        pltpu.make_async_copy(out_v.at[r * hbk:(r + 1) * hbk, :], out_hbm.at[r * hbk:(r + 1) * hbk, :], sem_o.at[r]).wait()

    def patch(g, sem):
        grow = rows + g
        cur = _ld(out_v, g, 16).astype(_F32)
        new = jnp.where(grow == i1s, res[0:1], jnp.where(grow == i2s, res[1:2], cur))
        _st(out_v, g, new)
        rs = pl.ds(pl.multiple_of(g // 2, 8), 8)
        return pltpu.make_async_copy(out_v.at[rs, :], out_hbm.at[rs, :], sem)

    g1 = pl.multiple_of((i1s // 16) * 16, 16)
    g2 = pl.multiple_of((i2s // 16) * 16, 16)
    c1 = patch(g1, sem_o.at[0])
    c1.start()

    @pl.when(g2 != g1)
    def _():
        c2 = patch(g2, sem_o.at[1])
        c2.start()
        c2.wait()

    c1.wait()


@jax.jit
def pallas_sequential_preLN__compressed_kv_cla__moe_arch_mod__prompt_kernel(A_x, A_c_kv, A_w_q, A_w_uk, A_w_uv, A_w_o, B_x, B_w_r, B_w_gate, B_w_up, B_w_down):
    hbm = pl.BlockSpec(memory_space=pl.ANY)
    vm = pltpu.VMEM
    u32 = jnp.uint32
    out = pl.pallas_call(
        _kernel,
        out_shape=jax.ShapeDtypeStruct((_S, _M), _BF16),
        in_specs=[hbm] * 6 + [pl.BlockSpec(memory_space=pltpu.VMEM)] + [hbm] * 3,
        out_specs=hbm,
        scratch_shapes=[
            vm((_S // 2, _M), u32), vm((_S // 2, _DC), u32), vm((_S // 2, _M), u32),
            vm((_NP, _M, _D), u32), vm((_NP, _DC, _D), u32), vm((_NP, _DC, _D), u32),
            vm((_H * _D // 2, _M), u32), vm((_M // 2, _F), u32), vm((_M // 2, _F), u32), vm((_F // 2, _M), u32),
            vm((_M // 2, 2 * _D), u32), vm((_DC // 2, 2 * _D), u32), vm((_DC // 2, 2 * _D), u32),
            vm((2, _S // 2, 2 * _D), u32), vm((2, _S // 2, 2 * _D), u32), vm((2, _S // 2, 2 * _D), u32),
            vm((_NP, _S // 2, 2 * _D), u32), vm((_S // 2, _M), u32), vm((_S // _RB, 8, _RB), _F32),
            vm((2, _RB, _M), _F32), vm((_RB, 128), _F32),
            pltpu.SemaphoreType.DMA((6,)), pltpu.SemaphoreType.DMA((3, _NP)), pltpu.SemaphoreType.DMA((_S // _RB,)), pltpu.SemaphoreType.DMA((8,)), pltpu.SemaphoreType.DMA((8,)),
        ],
        compiler_params=pltpu.CompilerParams(vmem_limit_bytes=120 * 2**20, flags={'XLA_TPU_EVENLY_DISTRIBUTE_CRITICAL_NODES': True}),
    )(A_x.reshape(_S, _M), A_c_kv.reshape(_S, _DC), A_w_q, A_w_uk, A_w_uv,
      A_w_o.reshape(_H * _D, _M), B_w_r.reshape(1, _M), B_w_gate, B_w_up, B_w_down)
    return out.reshape(1, _S, _M)
```

```python
import numpy as np
import jax
import jax.numpy as jnp
import jax.experimental.pallas as pl
import jax.experimental.pallas.tpu as pltpu

_S, _M, _H, _D, _DC, _F = 2048, 1024, 32, 128, 512, 3584
_NP = _H // 2
_BQ = 128
_RC = 512
_XC = 256
_RB = 256
_EC = 4
_SKEW = 3
_PPOS = (15, 15, 15, 15, 15, 15, 25, 27, 29, 31, 32, 32)
_EPS = 1e-5
_NT = (((1,), (1,)), ((), ()))


def _rows(r0, rows):
    h = rows // 2
    return pl.ds(r0 // 2, h) if isinstance(r0, int) else pl.ds(pl.multiple_of(r0 // 2, h), h)


def _ld(ref, r0, rows, cols=slice(None), lead=None):
    rs = _rows(r0, rows)
    v = ref[rs, cols] if lead is None else ref[lead, rs, cols]
    return pltpu.bitcast(v, jnp.bfloat16)


def _st(ref, r0, val, cols=slice(None), lead=None):
    rs = _rows(r0, val.shape[0])
    v = pltpu.bitcast(val.astype(jnp.bfloat16), jnp.uint32)
    if lead is None:
        ref[rs, cols] = v
    else:
        ref[lead, rs, cols] = v


def _lo(w):
    return pltpu.bitcast(w << 16, jnp.float32)


def _hi(w):
    return pltpu.bitcast(w & np.uint32(0xFFFF0000), jnp.float32)


def _unpack_pair(w):
    both = jnp.concatenate([_lo(w).astype(jnp.bfloat16), _hi(w).astype(jnp.bfloat16)], axis=1)
    return pltpu.bitcast(both, jnp.uint32)


def _recip(l):
    r = pl.reciprocal(l, approx=True)
    return r + r * (1.0 - l * r)


def _rb(v):
    return v.astype(jnp.bfloat16).astype(jnp.float32)


def _mm(a, b):
    return jnp.dot(a, b, preferred_element_type=jnp.float32)


def _schedule():
    nq, nr = _S // _BQ, _S // _RC
    proj = [(kind, r) for kind in "kvq" for r in range(nr)]
    att = [("a", hh, qb) for hh in range(2) for qb in reversed(range(nq))]
    out = []
    for j in range(len(att) + 1):
        if j == len(att):
            out.append(("f",))
        out += [p for p, at in zip(proj, _PPOS) if at == j]
        if j < len(att):
            out.append(att[j])
    return out


def _kernel(x_hbm, ckv_hbm, wq_hbm, wk_hbm, wv_hbm, wo_hbm, wr_ref, wg_hbm, wu_hbm, wd_hbm,
            out_hbm,
            x_v, ckv_v, ln_v, wq_v, wk_v, wv_v, wo_v, wg_v, wu_v, wd_v,
            wqb, wkb, wvb, q_v, k_v, v_v, ctx_v, out_v, r_v, acc_v, rr_v,
            sem_a, sem_w, sem_o, sem_x, sem_k):
    (x_hbm, ckv_hbm, wq_hbm, wk_hbm, wv_hbm, wo_hbm, wg_hbm, wu_hbm, wd_hbm, out_hbm) = [
        t.bitcast(jnp.uint32)
        for t in (x_hbm, ckv_hbm, wq_hbm, wk_hbm, wv_hbm, wo_hbm, wg_hbm, wu_hbm, wd_hbm, out_hbm)]
    nkc, nxc, nb = _S // _RC, _S // _XC, _S // _RB
    f32 = jnp.float32
    qscale = np.float32(_D ** -0.5 * np.log2(np.e))

    def cp_ck(c):
        rs = _rows(c * _RC, _RC)
        return pltpu.make_async_copy(ckv_hbm.at[rs], ckv_v.at[rs], sem_k.at[c])

    def cp_x(c):
        rs = _rows(c * _XC, _XC)
        return pltpu.make_async_copy(x_hbm.at[rs], x_v.at[rs], sem_x.at[c])

    def cp_pair(i):
        return [pltpu.make_async_copy(src.at[:, i, :], dst.at[i], sem_w.at[j, i])
                for j, (src, dst) in enumerate(((wk_hbm, wk_v), (wv_hbm, wv_v), (wq_hbm, wq_v)))]

    def cp_out(r):
        rs = _rows(r * _RB, _RB)
        return pltpu.make_async_copy(out_v.at[rs], out_hbm.at[rs], sem_o.at[r])

    cp_wo, cp_wg, cp_wu, cp_wd = [
        pltpu.make_async_copy(src, dst, sem_a.at[j])
        for j, (src, dst) in enumerate(((wo_hbm, wo_v), (wg_hbm, wg_v), (wu_hbm, wu_v), (wd_hbm, wd_v)))]

    def proj(kind, r, slot):
        r0 = r * _RC
        if kind == "k":
            _st(k_v, r0, _mm(_ld(ckv_v, r0, _RC), _ld(wkb, 0, _DC)), lead=slot)
        elif kind == "v":
            _st(v_v, r0, _mm(_ld(ckv_v, r0, _RC), _ld(wvb, 0, _DC)), lead=slot)
        else:
            _st(q_v, r0, _mm(_ld(ln_v, r0, _RC), _ld(wqb, 0, _M)) * qscale, lead=slot)

    def scores(slot, hh, qb):
        hs = slice(hh * _D, (hh + 1) * _D)
        n = (qb + 1) * _BQ
        ri = jax.lax.broadcasted_iota(jnp.int32, (_BQ, _BQ), 0)
        ci = jax.lax.broadcasted_iota(jnp.int32, (_BQ, _BQ), 1)
        s = jax.lax.dot_general(_ld(q_v, qb * _BQ, _BQ, hs, slot), _ld(k_v, 0, n, hs, slot), _NT,
                                preferred_element_type=f32)
        sd = jnp.where(ci <= ri, s[:, n - _BQ:], -1e9)
        s = jnp.concatenate([s[:, :n - _BQ], sd], axis=1) if qb > 0 else sd
        return s, jnp.max(s, axis=1, keepdims=True)

    def finish(i, slot, hh, qb, s, m):
        hs = slice(hh * _D, (hh + 1) * _D)
        p = jnp.exp2(s - m).astype(jnp.bfloat16)
        l = jnp.sum(p.astype(f32), axis=1, keepdims=True)
        o = _mm(p, _ld(v_v, 0, (qb + 1) * _BQ, hs, slot))
        _st(ctx_v, qb * _BQ, o * _recip(l), hs, i)

    def run(ops, i, slot):
        pend = []
        for op in ops:
            if op[0] == "a":
                pend.append(op[1:] + scores(slot, *op[1:]))
                if len(pend) > _SKEW:
                    finish(i, slot, *pend.pop(0))
            elif op[0] == "f":
                while pend:
                    finish(i, slot, *pend.pop(0))
            else:
                proj(op[0], op[1], 1 - slot)

    def ln1(c):
        xf = _ld(x_v, c * _XC, _XC).astype(f32)
        d = xf - jnp.mean(xf, axis=1, keepdims=True)
        var = jnp.mean(d * d, axis=1, keepdims=True)
        _st(ln_v, c * _XC, d * jax.lax.rsqrt(var + _EPS))

    def q0(c):
        _st(q_v, c * _XC, _mm(_ld(ln_v, c * _XC, _XC), _ld(wqb, 0, _M)) * qscale, lead=0)

    first = cp_pair(0)
    for cp in first[:2] + [cp_ck(c) for c in range(nkc)] + first[2:] + [cp_x(c) for c in range(nxc)]:
        cp.start()
    first[0].wait()
    first[1].wait()
    wkb[...] = _unpack_pair(wk_v[0])
    wvb[...] = _unpack_pair(wv_v[0])

    def kv_body(c, carry):
        cp_ck(c).wait()
        proj("k", c, 0)
        proj("v", c, 0)
        return carry

    jax.lax.fori_loop(0, nkc - 1, kv_body, 0)
    cp_ck(nkc - 1).wait()
    first[2].wait()
    cp_x(0).wait()
    proj("k", nkc - 1, 0)
    proj("v", nkc - 1, 0)
    wqb[...] = _unpack_pair(wq_v[0])
    ln1(0)

    def q_body(c, carry):
        cp_x(c + 1).wait()
        q0(c)
        ln1(c + 1)
        return carry

    jax.lax.fori_loop(0, nxc - 1, q_body, 0)
    for cp in cp_pair(1):
        cp.start()
    q0(nxc - 1)

    sched = _schedule()

    def pair_body(i, carry):
        @pl.when(i == 0)
        def _():
            for t in range(2, _NP):
                for cp in cp_pair(t):
                    cp.start()
            for cp in (cp_wo, cp_wg, cp_wu, cp_wd):
                cp.start()

        for cp in cp_pair(i + 1):
            cp.wait()
        wkb[...] = _unpack_pair(wk_v[i + 1])
        wvb[...] = _unpack_pair(wv_v[i + 1])
        wqb[...] = _unpack_pair(wq_v[i + 1])
        run(sched, i, i % 2)
        return carry

    jax.lax.fori_loop(0, _NP - 1, pair_body, 0)
    run([op for op in sched if op[0] in "af"], _NP - 1, (_NP - 1) % 2)

    cp_wo.wait()
    wr = wr_ref[...].astype(f32).reshape(1, _M)

    def epi(r, slot, c, nc):
        cr = _RB // nc
        r0 = r * _RB + c * cr
        h = _rb(_ld(x_v, r0, cr).astype(f32) + acc_v[slot, c * cr:(c + 1) * cr, :])
        d = h - jnp.mean(h, axis=1, keepdims=True)
        var = _rb(jnp.mean(d * d, axis=1, keepdims=True))
        ln = _rb(d * (1.0 / _rb(jnp.sqrt(_rb(var + _EPS)))))
        _st(ln_v, r0, ln)
        _st(x_v, r0, h)
        _st(out_v, r0, h + ln)
        rr = _rb(jnp.sum(ln * wr, axis=1, keepdims=True))
        rr_v[c * cr:(c + 1) * cr, :] = jnp.broadcast_to(rr, (cr, 128))

    def o_body(j, carry):
        r = jnp.maximum(j - 1, 0)
        acc = None
        per = _NP // _EC
        for i in range(_NP):
            t = _mm(_ld(ctx_v, j * _RB, _RB, lead=i), _ld(wo_v, i * 2 * _D, 2 * _D))
            acc = t if acc is None else acc + t
            if (i + 1) % per == per // 2:
                epi(r, 1 - j % 2, i // per, _EC)
        acc_v[j % 2] = acc
        r_v[r] = jnp.transpose(rr_v[...])[0:8, :]

        @pl.when(j > 0)
        def _():
            cp_out(r).start()
        return carry

    acc_v[1] = jnp.zeros((_RB, _M), f32)
    jax.lax.fori_loop(0, nb, o_body, 0)
    epi(nb - 1, (nb - 1) % 2, 0, 1)
    r_v[nb - 1] = jnp.transpose(rr_v[...])[0:8, :]
    cp_out(nb - 1).start()

    score = jnp.concatenate([r_v[j] for j in range(nb)], axis=1)
    idx = jax.lax.broadcasted_iota(jnp.int32, (8, _S), 1)
    m1 = jnp.max(score, axis=1, keepdims=True)
    i1 = jnp.min(jnp.where(score == m1, idx, _S), axis=1, keepdims=True)
    rest = jnp.where(idx == i1, -jnp.inf, score)
    m2 = jnp.max(rest, axis=1, keepdims=True)
    i2 = jnp.min(jnp.where((rest == m2) & (idx != i1), idx, _S), axis=1, keepdims=True)
    i1s = jnp.clip(jnp.max(i1), 0, _S - 1)
    i2s = jnp.clip(jnp.max(i2), 0, _S - 1)
    rows = jax.lax.broadcasted_iota(jnp.int32, (16, 1), 0)

    def two_rows(ref):
        def row(i):
            w = ref[pl.ds(i // 2, 1), :]
            return pltpu.bitcast(jnp.where(i % 2 == 0, w << 16, w & np.uint32(0xFFFF0000)), f32)
        return jnp.where(rows == 0, row(i1s), jnp.where(rows == 1, row(i2s), 0.0))

    xs = two_rows(ln_v)
    xb = xs.astype(jnp.bfloat16)
    cp_wg.wait()
    cp_wu.wait()
    cp_wd.wait()
    g = _rb(_mm(xb, _ld(wg_v, 0, _M)))
    u = _rb(_mm(xb, _ld(wu_v, 0, _M)))
    g = _rb(g * jax.nn.sigmoid(g))
    y = _rb(_mm((g * u).astype(jnp.bfloat16), _ld(wd_v, 0, _F)))
    y = _rb(y * _rb(jax.nn.sigmoid(jnp.where(rows == 0, m1[0:1, :], m2[0:1, :]))))
    res = two_rows(x_v) + _rb(xs + y)

    for r in range(nb):
        cp_out(r).wait()

    def patch(g0, sem):
        grow = rows + g0
        cur = _ld(out_v, g0, 16).astype(f32)
        _st(out_v, g0, jnp.where(grow == i1s, res[0:1], jnp.where(grow == i2s, res[1:2], cur)))
        rs = _rows(g0, 16)
        return pltpu.make_async_copy(out_v.at[rs], out_hbm.at[rs], sem)

    g1 = (i1s // 16) * 16
    g2 = (i2s // 16) * 16
    c1 = patch(g1, sem_o.at[0])
    c1.start()

    @pl.when(g2 != g1)
    def _():
        c2 = patch(g2, sem_o.at[1])
        c2.start()
        c2.wait()

    c1.wait()


@jax.jit
def pallas_sequential_preLN__compressed_kv_cla__moe_arch_mod__prompt_kernel(A_x, A_c_kv, A_w_q, A_w_uk, A_w_uv, A_w_o, B_x, B_w_r, B_w_gate, B_w_up, B_w_down):
    del B_x
    hbm = pl.BlockSpec(memory_space=pl.ANY)
    u32, f32 = jnp.uint32, jnp.float32
    vm = pltpu.VMEM
    dma = pltpu.SemaphoreType.DMA
    hd = 2 * _D
    out = pl.pallas_call(
        _kernel,
        out_shape=jax.ShapeDtypeStruct((_S, _M), jnp.bfloat16),
        in_specs=[hbm] * 6 + [pl.BlockSpec(memory_space=pltpu.VMEM)] + [hbm] * 3,
        out_specs=hbm,
        scratch_shapes=[
            vm((_S // 2, _M), u32), vm((_S // 2, _DC), u32), vm((_S // 2, _M), u32),
            vm((_NP, _M, _D), u32), vm((_NP, _DC, _D), u32), vm((_NP, _DC, _D), u32),
            vm((_H * _D // 2, _M), u32), vm((_M // 2, _F), u32), vm((_M // 2, _F), u32), vm((_F // 2, _M), u32),
            vm((_M // 2, hd), u32), vm((_DC // 2, hd), u32), vm((_DC // 2, hd), u32),
            vm((2, _S // 2, hd), u32), vm((2, _S // 2, hd), u32), vm((2, _S // 2, hd), u32),
            vm((_NP, _S // 2, hd), u32), vm((_S // 2, _M), u32), vm((_S // _RB, 8, _RB), f32),
            vm((2, _RB, _M), f32), vm((_RB, 128), f32),
            dma((4,)), dma((3, _NP)), dma((_S // _RB,)), dma((_S // _XC,)), dma((_S // _RC,)),
        ],
        compiler_params=pltpu.CompilerParams(
            vmem_limit_bytes=120 * 2**20,
            flags={"XLA_TPU_EVENLY_DISTRIBUTE_CRITICAL_NODES": True}),
    )(A_x.reshape(_S, _M), A_c_kv.reshape(_S, _DC), A_w_q, A_w_uk, A_w_uv,
      A_w_o.reshape(_H * _D, _M), B_w_r, B_w_gate, B_w_up, B_w_down)
    return out.reshape(1, _S, _M)
```
